```python
import jax
import jax.numpy as jnp

def _softmax(x, axis=-1):
    return jax.nn.softmax(x, axis=axis)

def _gelu(x):
    return jax.nn.gelu(x, approximate=True)

def _silu(x):
    return jax.nn.silu(x)

def _sigmoid(x):
    return jax.nn.sigmoid(x)

def _layernorm(x, axis=-1, eps=1e-05):
    m = jnp.mean(x, axis=axis, keepdims=True)
    v = jnp.var(x, axis=axis, keepdims=True)
    return (x - m) / jnp.sqrt(v + eps)

def _scatter_add(tgt, idx, src, axis=0):
    return tgt.at[idx].add(src)

def _segment_sum(src, seg, n):
    return jax.ops.segment_sum(src, seg, n)

class _Rng:

    def __init__(self, key):
        self._k = key

    def _next(self):
        self._k, sub = jax.random.split(self._k)
        return sub

    def normal(self, shape):
        return jax.random.normal(self._next(), shape, dtype=jnp.bfloat16)

    def randint(self, lo, hi, shape):
        return jax.random.randint(self._next(), shape, lo, hi, dtype=jnp.int32)

    def uniform(self, shape, lo=0.0, hi=1.0):
        return jax.random.uniform(self._next(), shape, jnp.bfloat16, lo, hi)

    def permutation(self, n):
        return jax.random.permutation(self._next(), n)
kernel_name = 'standalone__dilated_atrous__vision'

def setup_inputs():
    _rng = _Rng(jax.random.key(int.from_bytes(__import__("os").urandom(4), "little")))
    _w = lambda a: (lambda t: t.astype(jnp.bfloat16) if jnp.issubdtype(t.dtype, jnp.floating) else t)(jnp.asarray(a))
    H = W = 384
    C = 384
    k = 1
    return {'x': _w((lambda *s: _rng.normal(s) * 0.05)(1, H, W, C)), 'w': _w((lambda *s: _rng.normal(s) * 0.05)(k, k, C, C) * (1.0 / (k * C ** 0.5)))}

def reference(x, w):
    B, H, W, C = x.shape
    k = 1
    rate = 2
    pad = (k - 1) * rate // 2
    xp = jnp.pad(x, ((0, 0), (pad, pad), (pad, pad), (0, 0)))
    out = jnp.zeros_like(x)
    for i in range(k):
        for j in range(k):
            tap = xp[:, i * rate:i * rate + H, j * rate:j * rate + W, :].copy()
            out = out + jnp.einsum('bhwc,co->bhwo', tap, w[i, j])
    return out
```

```python
import jax
import jax.numpy as jnp
from jax import lax
import jax.experimental.pallas as pl
import jax.experimental.pallas.tpu as pltpu

_SLABS, _GROUPS, _GROUP_TILES = 36, 16, 32
_PIECE = 128
_EARLY = (0, 1, 5, 6, 10, 11, 12)
_LARGE = _EARLY + (2, 3, 4, 7)
_SMALL = (8, 9, 13, 14, 15)
_LATE, _LATE_RUN = (2, 7, 13), 3
_STEP_SLABS = 4
_STORES = (5, 5, 2)
_UP_FRONT = 4
_IDLE_NS = 126
_PAD_NS = 140
_TAIL = 12

_W_ROWS_TOTAL = 4096
_W_SLABS, _W_ROWS = 6, 64
_W_EARLY = 1280
_W_FIRST = 12
_W_PER_STEP = 20


def _lookup(table, i):
    words = [sum(v << 4 * n for n, v in enumerate(part)) for part in (table[:7], table[7:])]
    word = jnp.where(i < 7, words[0], words[1])
    return lax.shift_right_logical(word, 4 * jnp.where(i < 7, i, i - 7)) & 15


def _tile(r, c):
    return pl.ds(8 * (3 * r + c), 8)


@jax.jit
def pallas_standalone__dilated_atrous__vision_kernel(
    x: jax.Array,
    w: jax.Array,
):
    B, H, W, C = x.shape
    M = B * H * W
    group_rows = 3 * 8 * _GROUP_TILES
    assert w.shape == (1, 1, C, C) and C == 3 * 128
    assert M == _SLABS * _GROUPS * 8 * _GROUP_TILES
    assert sorted(_LARGE + _SMALL) == list(range(_GROUPS))
    assert sorted(_EARLY + tuple(i + k for i in _LATE for k in range(_LATE_RUN))) == list(range(_GROUPS))

    pieces = group_rows // _PIECE
    small = [(i, 2 * j) for i in _SMALL for j in range(pieces // 2)]
    early_steps = len(_EARLY) * _SLABS // _STEP_SLABS
    idle_slots = 2 * _SLABS - early_steps
    n_large = len(_LARGE) - 1
    assert len(small) == len(_STORES) + sum(_STORES) and idle_slots >= 0
    assert n_large - _UP_FRONT == len(_EARLY) - 1

    w_slabs = 3 * _SLABS
    w_sets = w_slabs // _W_SLABS
    assert w_slabs * _W_ROWS_TOTAL == _SLABS * _GROUPS * group_rows
    assert all((u * _W_ROWS_TOTAL + r) // group_rows in _EARLY
               for u in range(3) for r in range(0, _W_EARLY, 8))
    early_writes = w_sets * (_W_EARLY // _W_ROWS)
    set_writes = (_W_ROWS_TOTAL - _W_EARLY) // _W_ROWS
    late_steps = w_sets * len(_LATE)
    assert _W_FIRST <= early_writes
    assert all(_W_FIRST + (n + 1) * _W_PER_STEP <= early_writes + n // len(_LATE) * set_writes
               for n in range(late_steps))
    n_writes = early_writes + w_sets * set_writes

    def kernel_function(x_hbm, w_hbm, o_hbm, buf, wbuf):
        zero = jnp.int32(0)

        def load(groups, c):
            return jnp.concatenate(
                [buf[s, i, _tile(r, c)] for s, i in groups for r in range(_GROUP_TILES)], axis=0)

        def store(groups, c, res, lo, hi):
            for u in range(lo, hi):
                s, i = groups[u // _GROUP_TILES]
                buf[s, i, _tile(u % _GROUP_TILES, c)] = res[8 * u:8 * u + 8]

        def dot(a, b):
            return jnp.dot(a, b, preferred_element_type=jnp.float32).astype(buf.dtype)

        def run(out_sem):
            buf_w = buf.reshape(w_slabs, _W_ROWS_TOTAL, 128)
            out_w = o_hbm.reshape(w_slabs, _W_ROWS_TOTAL, 128)

            def start_write(pos):
                s, r, lo, hi = pos
                idx = (pl.ds(s, _W_SLABS), pl.ds(pl.multiple_of(r, _W_ROWS), _W_ROWS))
                pltpu.make_async_copy(buf_w.at[idx], out_w.at[idx], out_sem).start(priority=1)
                r = r + _W_ROWS
                set_done = r == hi
                s = jnp.where(set_done, s + _W_SLABS, s)
                pass_done = s == w_slabs
                lo = jnp.where(pass_done, hi, lo)
                hi = jnp.where(pass_done, _W_ROWS_TOTAL, hi)
                return jnp.where(pass_done, 0, s), jnp.where(set_done, lo, r), lo, hi

            def start_writes(count, pos):
                return lax.fori_loop(0, count, lambda _, pos: start_write(pos), pos)

            def read_phase(large_sems, sems):
                def read(idx, sem):
                    return pltpu.make_async_copy(x_hbm.at[idx], buf.at[idx], sem)

                def piece(j):
                    return pl.ds(j * _PIECE, _PIECE)

                def start_large(t):
                    i = _lookup(_LARGE, t)
                    for j in range(pieces):
                        read((slice(None), i, piece(j)), large_sems.at[t]).start(priority=1)

                def wait_large(t):
                    read((slice(None), _lookup(_LARGE, t)), large_sems.at[t]).wait()

                def start_small(n, u):
                    i, j = small[u]
                    s = (n >> 1) + 2 * u
                    s = jnp.where(s >= _SLABS, s - _SLABS, s)
                    rows = pl.ds(pl.multiple_of((j + (n & 1)) * _PIECE, _PIECE), _PIECE)
                    read((s, i, rows), sems.at[1]).start()

                w_copy = pltpu.make_async_copy(w_hbm, wbuf, sems.at[0])
                last = [read((slice(None), _LARGE[-1], piece(j)), sems.at[2])
                        for j in range(pieces - 1)]
                last.append(read(
                    (pl.ds(0, _SLABS - _TAIL), _LARGE[-1], piece(pieces - 1)), sems.at[2]))
                tail = read(
                    (pl.ds(_SLABS - _TAIL, _TAIL), _LARGE[-1], piece(pieces - 1)), sems.at[3])

                w_copy.start()
                lax.fori_loop(0, _UP_FRONT, lambda t, _: start_large(t), None)

                def idle_slot(n, _):
                    for u in range(len(small)):
                        start_small(n, u)
                        pl.delay(_IDLE_NS)

                lax.fori_loop(0, idle_slots, idle_slot, None)
                w_copy.wait()

                def step(n, carry):
                    t, i, s0 = carry

                    @pl.when(s0 == 0)
                    def _():
                        @pl.when(t + _UP_FRONT < n_large)
                        def _():
                            start_large(t + _UP_FRONT)

                        @pl.when(t + _UP_FRONT == n_large)
                        def _():
                            for copy in last + [tail]:
                                copy.start(priority=1)

                        wait_large(t)

                    ids = iter(range(len(small)))
                    groups = [(s0 + g, i) for g in range(_STEP_SLABS)]
                    blocks = []
                    for c in range(3):
                        start_small(idle_slots + n, next(ids))
                        blocks.append(load(groups, c))
                    xv = jnp.concatenate(blocks, axis=1)
                    for c, stores in enumerate(_STORES):
                        res = dot(xv, wbuf[:, c * 128:(c + 1) * 128])
                        cuts = [p * _STEP_SLABS * _GROUP_TILES // stores for p in range(stores + 1)]
                        for lo, hi in zip(cuts, cuts[1:]):
                            start_small(idle_slots + n, next(ids))
                            store(groups, c, res, lo, hi)
                    pl.delay(_PAD_NS)

                    s0 = s0 + _STEP_SLABS
                    t = jnp.where(s0 == _SLABS, t + 1, t)
                    return t, _lookup(_LARGE, t), jnp.where(s0 == _SLABS, 0, s0)

                lax.fori_loop(0, early_steps, step, (zero, jnp.int32(_LARGE[0]), zero))

                lax.fori_loop(len(_EARLY), n_large, lambda t, _: wait_large(t), None)
                for copy in last:
                    copy.wait()
                pos = start_writes(_W_FIRST, (zero, zero, zero, jnp.int32(_W_EARLY)))
                tail.wait()
                read((slice(None), pl.ds(0, len(_SMALL))), sems.at[1]).wait()
                return pos

            pos = pl.run_scoped(
                read_phase,
                pltpu.SemaphoreType.DMA((n_large,)),
                pltpu.SemaphoreType.DMA((4,)),
            )

            def step(_, carry):
                pos, s0, q = carry
                for _ in range(_W_PER_STEP):
                    pos = start_write(pos)
                i = _lookup(_LATE, q)
                groups = [(s0 + a, i + b) for a in range(_W_SLABS // 3) for b in range(_LATE_RUN)]
                xv = jnp.concatenate([load(groups, c) for c in range(3)], axis=1)
                res = dot(xv, wbuf[...])
                for c in range(3):
                    store(groups, c, res[:, c * 128:(c + 1) * 128], 0, len(groups) * _GROUP_TILES)
                q = q + 1
                wrap = q == len(_LATE)
                return pos, jnp.where(wrap, s0 + _W_SLABS // 3, s0), jnp.where(wrap, 0, q)

            pos, _, _ = lax.fori_loop(0, late_steps, step, (pos, zero, zero))
            start_writes(n_writes - _W_FIRST - late_steps * _W_PER_STEP, pos)
            pltpu.make_async_copy(buf, o_hbm, out_sem).wait()

        pl.run_scoped(run, pltpu.SemaphoreType.DMA(()))

    shape = (_SLABS, _GROUPS, group_rows, 128)
    out = pl.pallas_call(
        kernel_function,
        in_specs=[
            pl.BlockSpec(memory_space=pl.ANY),
            pl.BlockSpec(memory_space=pl.ANY),
        ],
        out_specs=pl.BlockSpec(memory_space=pl.ANY),
        out_shape=jax.ShapeDtypeStruct(shape, x.dtype),
        scratch_shapes=[
            pltpu.VMEM(shape, x.dtype),
            pltpu.VMEM((C, C), w.dtype),
        ],
        compiler_params=pltpu.CompilerParams(
            vmem_limit_bytes=120 * 2**20, disable_bounds_checks=True),
    )(x.reshape(M // 8, 8, 3, 128).transpose(0, 2, 1, 3).reshape(shape), w.reshape(C, C))
    return out.reshape(M // 8, 3, 8, 128).transpose(0, 2, 1, 3).reshape(B, H, W, C)
```

```python
import jax
import jax.numpy as jnp
from jax import lax
import jax.experimental.pallas as pl
import jax.experimental.pallas.tpu as pltpu

_SLABS, _GROUPS, _GROUP_TILES = 36, 16, 32
_PIECE = 128
_EARLY = (0, 1, 5, 6, 10, 11, 12)
_LARGE = _EARLY + (2, 3, 4, 7)
_SMALL = (8, 9, 13, 14, 15)
_LATE, _LATE_RUN = (2, 7, 13), 3
_STEP_SLABS = 4
_STORES = (5, 5, 2)
_UP_FRONT = 4
_IDLE_SPINS = 21
_PAD_SPINS = 24
_TAIL = 12

_W_ROWS_TOTAL = 4096
_W_SLABS, _W_ROWS = 6, 64
_W_EARLY = 1280
_W_FIRST = 18
_W_PER_STEP = 20


def _lookup(table, i):
    words = [sum(v << 4 * n for n, v in enumerate(part)) for part in (table[:7], table[7:])]
    word = jnp.where(i < 7, words[0], words[1])
    return lax.shift_right_logical(word, 4 * jnp.where(i < 7, i, i - 7)) & 15


def _tile(r, c):
    return pl.ds(8 * (3 * r + c), 8)


@jax.jit
def pallas_standalone__dilated_atrous__vision_kernel(
    x: jax.Array,
    w: jax.Array,
):
    B, H, W, C = x.shape
    M = B * H * W
    group_rows = 3 * 8 * _GROUP_TILES
    assert w.shape == (1, 1, C, C) and C == 3 * 128
    assert M == _SLABS * _GROUPS * 8 * _GROUP_TILES
    assert sorted(_LARGE + _SMALL) == list(range(_GROUPS))
    assert sorted(_EARLY + tuple(i + k for i in _LATE for k in range(_LATE_RUN))) == list(range(_GROUPS))

    pieces = group_rows // _PIECE
    piece_order = [j + half for j in range(pieces // 2) for half in (0, pieces // 2)]
    small = [(i, 2 * j) for i in _SMALL for j in range(pieces // 2)]
    early_steps = len(_EARLY) * _SLABS // _STEP_SLABS
    idle_slots = 2 * _SLABS - early_steps
    n_large = len(_LARGE) - 1
    assert len(small) == len(_STORES) + sum(_STORES) and idle_slots >= 0
    assert n_large - _UP_FRONT == len(_EARLY) - 1

    w_slabs = 3 * _SLABS
    w_sets = w_slabs // _W_SLABS
    assert w_slabs * _W_ROWS_TOTAL == _SLABS * _GROUPS * group_rows
    assert all((u * _W_ROWS_TOTAL + r) // group_rows in _EARLY
               for u in range(3) for r in range(0, _W_EARLY, 8))
    early_writes = w_sets * (_W_EARLY // _W_ROWS)
    set_writes = (_W_ROWS_TOTAL - _W_EARLY) // _W_ROWS
    late_steps = w_sets * len(_LATE)
    assert _W_FIRST <= early_writes
    assert all(_W_FIRST + (n + 1) * _W_PER_STEP <= early_writes + n // len(_LATE) * set_writes
               for n in range(late_steps))
    n_writes = early_writes + w_sets * set_writes

    def kernel_function(x_hbm, w_hbm, o_hbm, buf, wbuf, tick):
        zero = jnp.int32(0)

        def spin(count):
            def body(i, _):
                tick[0] = i
            lax.fori_loop(0, count, body, None)

        def load(groups, c):
            return jnp.concatenate(
                [buf[s, i, _tile(r, c)] for s, i in groups for r in range(_GROUP_TILES)], axis=0)

        def store(groups, c, res, lo, hi):
            for u in range(lo, hi):
                s, i = groups[u // _GROUP_TILES]
                buf[s, i, _tile(u % _GROUP_TILES, c)] = res[8 * u:8 * u + 8]

        def dot(a, b):
            return jnp.dot(a, b, preferred_element_type=jnp.float32).astype(buf.dtype)

        def run(out_sem):
            buf_w = buf.reshape(w_slabs, _W_ROWS_TOTAL, 128)
            out_w = o_hbm.reshape(w_slabs, _W_ROWS_TOTAL, 128)

            def start_write(pos):
                s, r, lo, hi = pos
                idx = (pl.ds(s, _W_SLABS), pl.ds(pl.multiple_of(r, _W_ROWS), _W_ROWS))
                pltpu.make_async_copy(buf_w.at[idx], out_w.at[idx], out_sem).start(priority=1)
                r = r + _W_ROWS
                set_done = r == hi
                s = jnp.where(set_done, s + _W_SLABS, s)
                pass_done = s == w_slabs
                lo = jnp.where(pass_done, hi, lo)
                hi = jnp.where(pass_done, _W_ROWS_TOTAL, hi)
                return jnp.where(pass_done, 0, s), jnp.where(set_done, lo, r), lo, hi

            def start_writes(count, pos):
                return lax.fori_loop(0, count, lambda _, pos: start_write(pos), pos)

            def read_phase(large_sems, sems):
                def read(idx, sem):
                    return pltpu.make_async_copy(x_hbm.at[idx], buf.at[idx], sem)

                def piece(j):
                    return pl.ds(j * _PIECE, _PIECE)

                def start_large(t):
                    i = _lookup(_LARGE, t)
                    for j in piece_order:
                        read((slice(None), i, piece(j)), large_sems.at[t]).start(priority=1)

                def wait_large(t):
                    read((slice(None), _lookup(_LARGE, t)), large_sems.at[t]).wait()

                def start_small(n, u):
                    i, j = small[u]
                    s = (n >> 1) + 4 * (u % 2)
                    s = jnp.where(s >= _SLABS, s - _SLABS, s)
                    rows = pl.ds(pl.multiple_of((j + (n & 1)) * _PIECE, _PIECE), _PIECE)
                    read((s, i, rows), sems.at[1]).start()

                w_copy = pltpu.make_async_copy(w_hbm, wbuf, sems.at[0])
                last = [read((slice(None), _LARGE[-1], piece(j)), sems.at[2])
                        for j in range(pieces - 1)]
                last.append(read(
                    (pl.ds(0, _SLABS - _TAIL), _LARGE[-1], piece(pieces - 1)), sems.at[2]))
                tail = read(
                    (pl.ds(_SLABS - _TAIL, _TAIL), _LARGE[-1], piece(pieces - 1)), sems.at[3])

                w_copy.start()
                lax.fori_loop(0, _UP_FRONT, lambda t, _: start_large(t), None)

                def idle_slot(n, _):
                    for u in range(len(small)):
                        start_small(n, u)
                        spin(_IDLE_SPINS)

                lax.fori_loop(0, idle_slots, idle_slot, None)
                w_copy.wait()

                def step(n, carry):
                    t, i, s0 = carry

                    @pl.when(s0 == 0)
                    def _():
                        @pl.when(t + _UP_FRONT < n_large)
                        def _():
                            start_large(t + _UP_FRONT)

                        @pl.when(t + _UP_FRONT == n_large)
                        def _():
                            for copy in last + [tail]:
                                copy.start(priority=1)

                        wait_large(t)

                    ids = iter(range(len(small)))
                    groups = [(s0 + g, i) for g in range(_STEP_SLABS)]
                    blocks = []
                    for c in range(3):
                        start_small(idle_slots + n, next(ids))
                        blocks.append(load(groups, c))
                    xv = jnp.concatenate(blocks, axis=1)
                    for c, stores in enumerate(_STORES):
                        res = dot(xv, wbuf[:, c * 128:(c + 1) * 128])
                        cuts = [p * _STEP_SLABS * _GROUP_TILES // stores for p in range(stores + 1)]
                        for lo, hi in zip(cuts, cuts[1:]):
                            start_small(idle_slots + n, next(ids))
                            store(groups, c, res, lo, hi)
                    spin(_PAD_SPINS)

                    s0 = s0 + _STEP_SLABS
                    t = jnp.where(s0 == _SLABS, t + 1, t)
                    return t, _lookup(_LARGE, t), jnp.where(s0 == _SLABS, 0, s0)

                lax.fori_loop(0, early_steps, step, (zero, jnp.int32(_LARGE[0]), zero))

                lax.fori_loop(len(_EARLY), n_large, lambda t, _: wait_large(t), None)
                for copy in last:
                    copy.wait()
                pos = start_writes(_W_FIRST, (zero, zero, zero, jnp.int32(_W_EARLY)))
                tail.wait()
                read((slice(None), pl.ds(0, len(_SMALL))), sems.at[1]).wait()
                return pos

            pos = pl.run_scoped(
                read_phase,
                pltpu.SemaphoreType.DMA((n_large,)),
                pltpu.SemaphoreType.DMA((4,)),
            )

            def step(_, carry):
                pos, s0, q = carry
                for _ in range(_W_PER_STEP):
                    pos = start_write(pos)
                i = _lookup(_LATE, q)
                groups = [(s0 + a, i + b) for a in range(_W_SLABS // 3) for b in range(_LATE_RUN)]
                xv = jnp.concatenate([load(groups, c) for c in range(3)], axis=1)
                res = dot(xv, wbuf[...])
                for c in range(3):
                    store(groups, c, res[:, c * 128:(c + 1) * 128], 0, len(groups) * _GROUP_TILES)
                q = q + 1
                wrap = q == len(_LATE)
                return pos, jnp.where(wrap, s0 + _W_SLABS // 3, s0), jnp.where(wrap, 0, q)

            pos, _, _ = lax.fori_loop(0, late_steps, step, (pos, zero, zero))
            start_writes(n_writes - _W_FIRST - late_steps * _W_PER_STEP, pos)
            pltpu.make_async_copy(buf, o_hbm, out_sem).wait()

        pl.run_scoped(run, pltpu.SemaphoreType.DMA(()))

    shape = (_SLABS, _GROUPS, group_rows, 128)
    out = pl.pallas_call(
        kernel_function,
        in_specs=[
            pl.BlockSpec(memory_space=pl.ANY),
            pl.BlockSpec(memory_space=pl.ANY),
        ],
        out_specs=pl.BlockSpec(memory_space=pl.ANY),
        out_shape=jax.ShapeDtypeStruct(shape, x.dtype),
        scratch_shapes=[
            pltpu.VMEM(shape, x.dtype),
            pltpu.VMEM((C, C), w.dtype),
            pltpu.SMEM((1,), jnp.int32),
        ],
        compiler_params=pltpu.CompilerParams(
            vmem_limit_bytes=120 * 2**20, disable_bounds_checks=True),
    )(x.reshape(M // 8, 8, 3, 128).transpose(0, 2, 1, 3).reshape(shape), w.reshape(C, C))
    return out.reshape(M // 8, 3, 8, 128).transpose(0, 2, 1, 3).reshape(B, H, W, C)
```

```python
import jax
import jax.numpy as jnp
from jax import lax
import jax.experimental.pallas as pl
import jax.experimental.pallas.tpu as pltpu

_SLABS, _GROUPS, _GROUP_TILES = 36, 16, 32
_PIECE = 128
_EARLY = (0, 1, 5, 6, 10, 11, 12)
_LARGE = _EARLY + (2, 3, 4, 7)
_SMALL = (range(8, 10), range(13, 16))
_LATE, _LATE_RUN = (2, 7, 13), 3
_STEP_SLABS = 4
_STORES = (5, 5, 2)
_UP_FRONT = 4
_IDLE_SPINS = 21
_PAD_SPINS = 22
_TAIL = 12

_W_ROWS_TOTAL = 4096
_W_SLABS, _W_ROWS = 6, 64
_W_EARLY = 1280
_W_FIRST = 18
_W_PER_STEP = 20


def _lookup(table, i):
    words = [sum(v << 4 * n for n, v in enumerate(part)) for part in (table[:7], table[7:])]
    word = jnp.where(i < 7, words[0], words[1])
    return lax.shift_right_logical(word, 4 * jnp.where(i < 7, i, i - 7)) & 15


def _tile(r, c):
    return pl.ds(8 * (3 * r + c), 8)


@jax.jit
def pallas_standalone__dilated_atrous__vision_kernel(
    x: jax.Array,
    w: jax.Array,
):
    B, H, W, C = x.shape
    M = B * H * W
    group_rows = 3 * 8 * _GROUP_TILES
    assert w.shape == (1, 1, C, C) and C == 3 * 128
    assert M == _SLABS * _GROUPS * 8 * _GROUP_TILES
    assert sorted(_LARGE + tuple(i for run in _SMALL for i in run)) == list(range(_GROUPS))
    assert sorted(_EARLY + tuple(i + k for i in _LATE for k in range(_LATE_RUN))) == list(range(_GROUPS))

    pieces = group_rows // _PIECE
    piece_order = [j + half for j in range(pieces // 2) for half in (0, pieces // 2)]
    small = [(k, i, 2 * j) for k, run in enumerate(_SMALL) for i in run for j in range(pieces // 2)]
    early_steps = len(_EARLY) * _SLABS // _STEP_SLABS
    idle_slots = 2 * _SLABS - early_steps
    n_large = len(_LARGE) - 1
    assert len(small) == len(_STORES) + sum(_STORES) and idle_slots >= 0
    assert n_large - _UP_FRONT == len(_EARLY) - 1

    w_slabs = 3 * _SLABS
    w_sets = w_slabs // _W_SLABS
    assert w_slabs * _W_ROWS_TOTAL == _SLABS * _GROUPS * group_rows
    assert all((u * _W_ROWS_TOTAL + r) // group_rows in _EARLY
               for u in range(3) for r in range(0, _W_EARLY, 8))
    early_writes = w_sets * (_W_EARLY // _W_ROWS)
    set_writes = (_W_ROWS_TOTAL - _W_EARLY) // _W_ROWS
    late_steps = w_sets * len(_LATE)
    assert _W_FIRST <= early_writes
    assert all(_W_FIRST + (n + 1) * _W_PER_STEP <= early_writes + n // len(_LATE) * set_writes
               for n in range(late_steps))
    n_writes = early_writes + w_sets * set_writes

    def kernel_function(x_hbm, w_hbm, o_hbm, buf, wbuf, tick):
        zero = jnp.int32(0)

        def spin(count):
            def body(i, _):
                tick[0] = i
            lax.fori_loop(0, count, body, None)

        def load(groups, c):
            return jnp.concatenate(
                [buf[s, i, _tile(r, c)] for s, i in groups for r in range(_GROUP_TILES)], axis=0)

        def store(groups, c, res, lo, hi):
            for u in range(lo, hi):
                s, i = groups[u // _GROUP_TILES]
                buf[s, i, _tile(u % _GROUP_TILES, c)] = res[8 * u:8 * u + 8]

        def dot(a, b):
            return jnp.dot(a, b, preferred_element_type=jnp.float32).astype(buf.dtype)

        def both_phases(out_sem):
            buf_w = buf.reshape(w_slabs, _W_ROWS_TOTAL, 128)
            out_w = o_hbm.reshape(w_slabs, _W_ROWS_TOTAL, 128)

            def start_write(pos):
                s, r, lo, hi = pos
                idx = (pl.ds(s, _W_SLABS), pl.ds(pl.multiple_of(r, _W_ROWS), _W_ROWS))
                pltpu.make_async_copy(buf_w.at[idx], out_w.at[idx], out_sem).start(priority=1)
                r = r + _W_ROWS
                set_done = r == hi
                s = jnp.where(set_done, s + _W_SLABS, s)
                pass_done = s == w_slabs
                lo = jnp.where(pass_done, hi, lo)
                hi = jnp.where(pass_done, _W_ROWS_TOTAL, hi)
                return jnp.where(pass_done, 0, s), jnp.where(set_done, lo, r), lo, hi

            def start_writes(count, pos):
                return lax.fori_loop(0, count, lambda _, pos: start_write(pos), pos)

            def read_phase(large_sems, small_sems, sems):
                def read(idx, sem):
                    return pltpu.make_async_copy(x_hbm.at[idx], buf.at[idx], sem)

                def piece(j):
                    return pl.ds(j * _PIECE, _PIECE)

                def start_large(t):
                    i = _lookup(_LARGE, t)
                    for j in piece_order:
                        read((slice(None), i, piece(j)), large_sems.at[t]).start(priority=1)

                def wait_large(t):
                    read((slice(None), _lookup(_LARGE, t)), large_sems.at[t]).wait()

                def start_small(n, u):
                    k, i, j = small[u]
                    s = (n >> 1) + 4 * (u % 2)
                    s = jnp.where(s >= _SLABS, s - _SLABS, s)
                    rows = pl.ds(pl.multiple_of((j + (n & 1)) * _PIECE, _PIECE), _PIECE)
                    read((s, i, rows), small_sems.at[k]).start()

                w_copy = pltpu.make_async_copy(w_hbm, wbuf, sems.at[0])
                last = [read((slice(None), _LARGE[-1], piece(j)), sems.at[1])
                        for j in range(pieces - 1)]
                last.append(read(
                    (pl.ds(0, _SLABS - _TAIL), _LARGE[-1], piece(pieces - 1)), sems.at[1]))
                tail = read(
                    (pl.ds(_SLABS - _TAIL, _TAIL), _LARGE[-1], piece(pieces - 1)), sems.at[2])

                w_copy.start()
                lax.fori_loop(0, _UP_FRONT, lambda t, _: start_large(t), None)

                def idle_slot(n, _):
                    for u in range(len(small)):
                        start_small(n, u)
                        spin(_IDLE_SPINS)

                lax.fori_loop(0, idle_slots, idle_slot, None)
                w_copy.wait()

                def step(n, carry):
                    t, i, s0 = carry

                    @pl.when(s0 == 0)
                    def _():
                        @pl.when(t + _UP_FRONT < n_large)
                        def _():
                            start_large(t + _UP_FRONT)

                        @pl.when(t + _UP_FRONT == n_large)
                        def _():
                            for copy in last + [tail]:
                                copy.start(priority=1)

                        wait_large(t)

                    ids = iter(range(len(small)))
                    groups = [(s0 + g, i) for g in range(_STEP_SLABS)]
                    blocks = []
                    for c in range(3):
                        start_small(idle_slots + n, next(ids))
                        blocks.append(load(groups, c))
                    xv = jnp.concatenate(blocks, axis=1)
                    for c, stores in enumerate(_STORES):
                        res = dot(xv, wbuf[:, c * 128:(c + 1) * 128])
                        cuts = [p * _STEP_SLABS * _GROUP_TILES // stores for p in range(stores + 1)]
                        for lo, hi in zip(cuts, cuts[1:]):
                            start_small(idle_slots + n, next(ids))
                            store(groups, c, res, lo, hi)
                    spin(_PAD_SPINS)

                    s0 = s0 + _STEP_SLABS
                    t = jnp.where(s0 == _SLABS, t + 1, t)
                    return t, _lookup(_LARGE, t), jnp.where(s0 == _SLABS, 0, s0)

                lax.fori_loop(0, early_steps, step, (zero, jnp.int32(_LARGE[0]), zero))

                lax.fori_loop(len(_EARLY), n_large, lambda t, _: wait_large(t), None)
                for copy in last:
                    copy.wait()
                pos = start_writes(_W_FIRST, (zero, zero, zero, jnp.int32(_W_EARLY)))
                tail.wait()
                for k, run in enumerate(_SMALL):
                    read((slice(None), pl.ds(run.start, len(run))), small_sems.at[k]).wait()
                return pos

            pos = pl.run_scoped(
                read_phase,
                pltpu.SemaphoreType.DMA((n_large,)),
                pltpu.SemaphoreType.DMA((len(_SMALL),)),
                pltpu.SemaphoreType.DMA((3,)),
            )

            def step(_, carry):
                pos, s0, q = carry
                for _ in range(_W_PER_STEP):
                    pos = start_write(pos)
                i = _lookup(_LATE, q)
                groups = [(s0 + a, i + b) for a in range(_W_SLABS // 3) for b in range(_LATE_RUN)]
                xv = jnp.concatenate([load(groups, c) for c in range(3)], axis=1)
                res = dot(xv, wbuf[...])
                for c in range(3):
                    store(groups, c, res[:, c * 128:(c + 1) * 128], 0, len(groups) * _GROUP_TILES)
                q = q + 1
                wrap = q == len(_LATE)
                return pos, jnp.where(wrap, s0 + _W_SLABS // 3, s0), jnp.where(wrap, 0, q)

            pos, _, _ = lax.fori_loop(0, late_steps, step, (pos, zero, zero))
            start_writes(n_writes - _W_FIRST - late_steps * _W_PER_STEP, pos)
            pltpu.make_async_copy(buf, o_hbm, out_sem).wait()

        pl.run_scoped(both_phases, pltpu.SemaphoreType.DMA(()))

    shape = (_SLABS, _GROUPS, group_rows, 128)
    out = pl.pallas_call(
        kernel_function,
        in_specs=[
            pl.BlockSpec(memory_space=pl.ANY),
            pl.BlockSpec(memory_space=pl.ANY),
        ],
        out_specs=pl.BlockSpec(memory_space=pl.ANY),
        out_shape=jax.ShapeDtypeStruct(shape, x.dtype),
        scratch_shapes=[
            pltpu.VMEM(shape, x.dtype),
            pltpu.VMEM((C, C), w.dtype),
            pltpu.SMEM((1,), jnp.int32),
        ],
        compiler_params=pltpu.CompilerParams(
            vmem_limit_bytes=120 * 2**20, disable_bounds_checks=True),
    )(x.reshape(M // 8, 8, 3, 128).transpose(0, 2, 1, 3).reshape(shape), w.reshape(C, C))
    return out.reshape(M // 8, 3, 8, 128).transpose(0, 2, 1, 3).reshape(B, H, W, C)
```

```python
import jax
import jax.numpy as jnp
from jax import lax
import jax.experimental.pallas as pl
import jax.experimental.pallas.tpu as pltpu

_SLABS, _SLAB_ROWS = 108, 4096
_PIECE = 128
_BAND = 36
_EARLY_PIECES = 18
_LARGE_PIECES = 22
_UP_FRONT = 26
_TAIL = 12
_W_SLABS, _W_ROWS = 6, 64
_W_EARLY = (512, 1792)
_W_FIRST = 18
_W_PER_STEP = 20

_GROUPS, _GROUP_TILES = 16, 32
_EARLY = (0, 11, 6, 1, 12, 7, 2)
_LATE, _LATE_RUN = (3, 8, 13), 3
_STEP_TRIPLES = 4
_STORES = (5, 5, 2)
_IDLE_SPINS = 21
_PAD_SPINS = 22


def _lookup(table, i):
    word = sum(v << 4 * n for n, v in enumerate(table))
    return lax.shift_right_logical(word, 4 * i) & 15


def _tile(r, c):
    return pl.ds(8 * (3 * r + c), 8)


@jax.jit
def pallas_standalone__dilated_atrous__vision_kernel(
    x: jax.Array,
    w: jax.Array,
):
    B, H, W, C = x.shape
    M = B * H * W
    group_rows = 3 * 8 * _GROUP_TILES
    assert w.shape == (1, 1, C, C) and C == 3 * 128
    triples = _SLABS // 3
    assert M == triples * _GROUPS * 8 * _GROUP_TILES
    assert _SLABS * _SLAB_ROWS == triples * _GROUPS * group_rows
    assert sorted(_EARLY + tuple(i + k for i in _LATE for k in range(_LATE_RUN))) == list(range(_GROUPS))

    bands = _SLABS // _BAND
    pieces = _SLAB_ROWS // _PIECE
    first_batch = _EARLY_PIECES - 2 * (len(_EARLY) - 1)
    assert all((i + 1) * group_rows // _PIECE % pieces == first_batch + 2 * k
               and i * group_rows // _SLAB_ROWS == ((i + 1) * group_rows - 1) // _SLAB_ROWS
               for k, i in enumerate(_EARLY))
    n_batches = bands * len(_EARLY)
    n_early = bands * _EARLY_PIECES
    assert (n_early - _UP_FRONT) % 2 == 0 and n_early - _UP_FRONT < 2 * n_batches
    band_triples = _BAND // 3
    early_steps = n_batches * band_triples // _STEP_TRIPLES

    small = [(band, j) for band in range(bands) for j in range(_LARGE_PIECES, pieces, 2)]
    idle_slots = 2 * _BAND - early_steps
    assert len(small) == len(_STORES) + sum(_STORES) and idle_slots >= 0

    w_sets = _SLABS // _W_SLABS
    assert all((u * _SLAB_ROWS + r) // group_rows in _EARLY
               for u in range(3) for r in range(*_W_EARLY, 8))
    early_writes = w_sets * ((_W_EARLY[1] - _W_EARLY[0]) // _W_ROWS)
    n_writes = w_sets * (_SLAB_ROWS // _W_ROWS)
    late_steps = w_sets * len(_LATE)
    assert _W_FIRST <= early_writes
    assert all(_W_FIRST + (n + 1) * _W_PER_STEP
               <= early_writes + n // len(_LATE) * ((n_writes - early_writes) // w_sets)
               for n in range(late_steps))

    def kernel_function(x_hbm, w_hbm, o_hbm, buf, wbuf, tick):
        zero = jnp.int32(0)

        def spin(count):
            def body(i, _):
                tick[0] = i
            lax.fori_loop(0, count, body, None)

        def load(groups, c):
            return jnp.concatenate(
                [buf[s, i, _tile(r, c)] for s, i in groups for r in range(_GROUP_TILES)], axis=0)

        def store(groups, c, res, lo, hi):
            for u in range(lo, hi):
                s, i = groups[u // _GROUP_TILES]
                buf[s, i, _tile(u % _GROUP_TILES, c)] = res[8 * u:8 * u + 8]

        def dot(a, b):
            return jnp.dot(a, b, preferred_element_type=jnp.float32).astype(buf.dtype)

        def both_phases(out_sem):
            x_slabs, buf_slabs, out_slabs = (
                ref.reshape(_SLABS, _SLAB_ROWS, 128) for ref in (x_hbm, buf, o_hbm))

            def start_write(pos):
                s, r, lo, hi = pos
                idx = (pl.ds(s, _W_SLABS), pl.ds(pl.multiple_of(r, _W_ROWS), _W_ROWS))
                pltpu.make_async_copy(
                    buf_slabs.at[idx], out_slabs.at[idx], out_sem).start(priority=1)
                r = (r + _W_ROWS) & (_SLAB_ROWS - 1)
                set_done = r == hi
                s = jnp.where(set_done, s + _W_SLABS, s)
                pass_done = s == _SLABS
                lo, hi = jnp.where(pass_done, hi, lo), jnp.where(pass_done, lo, hi)
                return jnp.where(pass_done, 0, s), jnp.where(set_done, lo, r), lo, hi

            def start_writes(count, pos):
                return lax.fori_loop(0, count, lambda _, pos: start_write(pos), pos)

            def read_phase(batch_sems, sems):
                def read(slabs, j, count, sem):
                    rows = pl.ds(pl.multiple_of(j * _PIECE, _PIECE), count * _PIECE)
                    return pltpu.make_async_copy(
                        x_slabs.at[slabs, rows], buf_slabs.at[slabs, rows], sem)

                def band_slabs(band):
                    return pl.ds(band * _BAND, _BAND)

                def band_of(e, per_band):
                    return sum((e >= b * per_band).astype(jnp.int32) for b in range(1, bands))

                def start_early(e):
                    band = band_of(e, _EARLY_PIECES)
                    j = e - band * _EARLY_PIECES
                    k = jnp.maximum(j - first_batch + 2, 0) >> 1
                    read(band_slabs(band), j, 1,
                         batch_sems.at[band * len(_EARLY) + k]).start(priority=1)

                def wait_batch(band, k):
                    sem = batch_sems.at[band * len(_EARLY) + k]

                    @pl.when(k == 0)
                    def _():
                        read(band_slabs(band), 0, first_batch, sem).wait()

                    @pl.when(k > 0)
                    def _():
                        read(band_slabs(band), first_batch + 2 * k - 2, 2, sem).wait()

                def start_small(n, u):
                    band, j = small[u]
                    s = (n >> 1) + 4 * (u % 2)
                    s = jnp.where(s >= _BAND, s - _BAND, s)
                    read(band * _BAND + s, j + (n & 1), 1, sems.at[1]).start()

                w_copy = pltpu.make_async_copy(w_hbm, wbuf, sems.at[0])
                last = [read(band_slabs(band), j, 1, sems.at[2])
                        for j in range(_EARLY_PIECES, _LARGE_PIECES) for band in range(bands)
                        if (j, band) != (_LARGE_PIECES - 1, bands - 1)]
                last.append(read(
                    pl.ds(_SLABS - _BAND, _BAND - _TAIL), _LARGE_PIECES - 1, 1, sems.at[2]))
                tail = read(pl.ds(_SLABS - _TAIL, _TAIL), _LARGE_PIECES - 1, 1, sems.at[3])

                w_copy.start()
                lax.fori_loop(0, _UP_FRONT, lambda e, _: start_early(e), None)

                def idle_slot(n, _):
                    for u in range(len(small)):
                        start_small(n, u)
                        spin(_IDLE_SPINS)

                lax.fori_loop(0, idle_slots, idle_slot, None)
                w_copy.wait()

                def step(n, carry):
                    band, k, s0, started = carry

                    @pl.when(s0 == 0)
                    def _():
                        @pl.when(started < n_early)
                        def _():
                            start_early(started)
                            start_early(started + 1)

                        @pl.when(started == n_early)
                        def _():
                            for copy in last + [tail]:
                                copy.start(priority=1)

                        wait_batch(band, k)

                    ids = iter(range(len(small)))
                    i = _lookup(_EARLY, k)
                    groups = [(band * band_triples + s0 + g, i) for g in range(_STEP_TRIPLES)]
                    blocks = []
                    for c in range(3):
                        start_small(idle_slots + n, next(ids))
                        blocks.append(load(groups, c))
                    xv = jnp.concatenate(blocks, axis=1)
                    for c, stores in enumerate(_STORES):
                        res = dot(xv, wbuf[:, c * 128:(c + 1) * 128])
                        cuts = [p * len(groups) * _GROUP_TILES // stores for p in range(stores + 1)]
                        for lo, hi in zip(cuts, cuts[1:]):
                            start_small(idle_slots + n, next(ids))
                            store(groups, c, res, lo, hi)
                    spin(_PAD_SPINS)

                    started = jnp.where(s0 == 0, started + 2, started)
                    s0 = s0 + _STEP_TRIPLES
                    batch_done = s0 == band_triples
                    k = jnp.where(batch_done, k + 1, k)
                    band_done = k == len(_EARLY)
                    return (jnp.where(band_done, band + 1, band), jnp.where(band_done, 0, k),
                            jnp.where(batch_done, 0, s0), started)

                lax.fori_loop(0, early_steps, step, (zero, zero, zero, jnp.int32(_UP_FRONT)))

                for copy in last:
                    copy.wait()
                lo, hi = map(jnp.int32, _W_EARLY)
                pos = start_writes(_W_FIRST, (zero, lo, lo, hi))
                tail.wait()
                read(slice(None), _LARGE_PIECES, pieces - _LARGE_PIECES,
                     sems.at[1]).wait()
                return pos

            pos = pl.run_scoped(
                read_phase,
                pltpu.SemaphoreType.DMA((n_batches,)),
                pltpu.SemaphoreType.DMA((4,)),
            )

            def step(_, carry):
                pos, s0, q = carry
                for _ in range(_W_PER_STEP):
                    pos = start_write(pos)
                i = _lookup(_LATE, q)
                groups = [(s0 + a, i + b) for a in range(_W_SLABS // 3) for b in range(_LATE_RUN)]
                xv = jnp.concatenate([load(groups, c) for c in range(3)], axis=1)
                res = dot(xv, wbuf[...])
                for c in range(3):
                    store(groups, c, res[:, c * 128:(c + 1) * 128], 0, len(groups) * _GROUP_TILES)
                q = q + 1
                wrap = q == len(_LATE)
                return pos, jnp.where(wrap, s0 + _W_SLABS // 3, s0), jnp.where(wrap, 0, q)

            pos, _, _ = lax.fori_loop(0, late_steps, step, (pos, zero, zero))
            start_writes(n_writes - _W_FIRST - late_steps * _W_PER_STEP, pos)
            pltpu.make_async_copy(buf, o_hbm, out_sem).wait()

        pl.run_scoped(both_phases, pltpu.SemaphoreType.DMA(()))

    shape = (triples, _GROUPS, group_rows, 128)
    out = pl.pallas_call(
        kernel_function,
        in_specs=[
            pl.BlockSpec(memory_space=pl.ANY),
            pl.BlockSpec(memory_space=pl.ANY),
        ],
        out_specs=pl.BlockSpec(memory_space=pl.ANY),
        out_shape=jax.ShapeDtypeStruct(shape, x.dtype),
        scratch_shapes=[
            pltpu.VMEM(shape, x.dtype),
            pltpu.VMEM((C, C), w.dtype),
            pltpu.SMEM((1,), jnp.int32),
        ],
        compiler_params=pltpu.CompilerParams(
            vmem_limit_bytes=120 * 2**20, disable_bounds_checks=True),
    )(x.reshape(M // 8, 8, 3, 128).transpose(0, 2, 1, 3).reshape(shape), w.reshape(C, C))
    return out.reshape(M // 8, 3, 8, 128).transpose(0, 2, 1, 3).reshape(B, H, W, C)
```

```python
import jax
import jax.numpy as jnp
from jax import lax
import jax.experimental.pallas as pl
import jax.experimental.pallas.tpu as pltpu

_SLABS, _SLAB_ROWS = 108, 4096
_PIECE = 128
_BAND = 36
_EARLY_PIECES = 18
_LARGE_PIECES = 22
_UP_FRONT = 26
_TAIL = 12
_W_SLABS, _W_ROWS = 6, 64
_W_EARLY = (512, 1792)
_W_FIRST = 18
_W_PER_STEP = 20

_GROUPS, _GROUP_TILES = 16, 32
_EARLY = (0, 11, 6, 1, 12, 7, 2)
_LATE, _LATE_RUN = (3, 8, 13), 3
_STEP_TRIPLES = 4
_STORES = (5, 5, 2)
_IDLE_SPINS = 21
_PAD_SPINS = 22


def _lookup(table, i):
    word = sum(v << 4 * n for n, v in enumerate(table))
    return lax.shift_right_logical(word, 4 * i) & 15


def _tile(r, c):
    return pl.ds(8 * (3 * r + c), 8)


@jax.jit
def pallas_standalone__dilated_atrous__vision_kernel(
    x: jax.Array,
    w: jax.Array,
):
    B, H, W, C = x.shape
    M = B * H * W
    group_rows = 3 * 8 * _GROUP_TILES
    assert w.shape == (1, 1, C, C) and C == 3 * 128
    triples = _SLABS // 3
    assert M == triples * _GROUPS * 8 * _GROUP_TILES
    assert _SLABS * _SLAB_ROWS == triples * _GROUPS * group_rows
    assert sorted(_EARLY + tuple(i + k for i in _LATE for k in range(_LATE_RUN))) == list(range(_GROUPS))

    bands = _SLABS // _BAND
    pieces = _SLAB_ROWS // _PIECE
    first_batch = _EARLY_PIECES - 2 * (len(_EARLY) - 1)
    assert all((i + 1) * group_rows // _PIECE % pieces == first_batch + 2 * k
               and i * group_rows // _SLAB_ROWS == ((i + 1) * group_rows - 1) // _SLAB_ROWS
               for k, i in enumerate(_EARLY))
    n_batches = bands * len(_EARLY)
    n_early = bands * _EARLY_PIECES
    assert (n_early - _UP_FRONT) % 2 == 0 and n_early - _UP_FRONT < 2 * n_batches
    band_triples = _BAND // 3
    early_steps = n_batches * band_triples // _STEP_TRIPLES

    small = [(band, j) for band in range(bands) for j in range(_LARGE_PIECES, pieces, 2)]
    idle_slots = 2 * _BAND - early_steps
    assert len(small) == len(_STORES) + sum(_STORES) and idle_slots >= 0

    w_sets = _SLABS // _W_SLABS
    assert all((u * _SLAB_ROWS + r) // group_rows in _EARLY
               for u in range(3) for r in range(*_W_EARLY, 8))
    early_writes = w_sets * ((_W_EARLY[1] - _W_EARLY[0]) // _W_ROWS)
    n_writes = w_sets * (_SLAB_ROWS // _W_ROWS)
    late_steps = w_sets * len(_LATE)
    assert _W_FIRST <= early_writes
    assert all(_W_FIRST + (n + 1) * _W_PER_STEP
               <= early_writes + n // len(_LATE) * ((n_writes - early_writes) // w_sets)
               for n in range(late_steps))

    def kernel_function(x_hbm, w_hbm, o_hbm, buf, wbuf, tick):
        zero = jnp.int32(0)

        def spin(count):
            def body(i, _):
                tick[0] = i
            lax.fori_loop(0, count, body, None)

        def load(groups, c):
            return jnp.concatenate(
                [buf[s, i, _tile(r, c)] for s, i in groups for r in range(_GROUP_TILES)], axis=0)

        def store(groups, c, res, lo, hi):
            for u in range(lo, hi):
                s, i = groups[u // _GROUP_TILES]
                buf[s, i, _tile(u % _GROUP_TILES, c)] = res[8 * u:8 * u + 8]

        def dot(a, b):
            return jnp.dot(a, b, preferred_element_type=jnp.float32).astype(buf.dtype)

        def both_phases(out_sem):
            x_slabs, buf_slabs, out_slabs = (
                ref.reshape(_SLABS, _SLAB_ROWS, 128) for ref in (x_hbm, buf, o_hbm))

            def start_write(pos):
                s, r, lo, hi = pos
                idx = (pl.ds(s, _W_SLABS), pl.ds(pl.multiple_of(r, _W_ROWS), _W_ROWS))
                pltpu.make_async_copy(
                    buf_slabs.at[idx], out_slabs.at[idx], out_sem).start(priority=1)
                r = (r + _W_ROWS) & (_SLAB_ROWS - 1)
                set_done = r == hi
                s = jnp.where(set_done, s + _W_SLABS, s)
                pass_done = s == _SLABS
                lo, hi = jnp.where(pass_done, hi, lo), jnp.where(pass_done, lo, hi)
                return jnp.where(pass_done, 0, s), jnp.where(set_done, lo, r), lo, hi

            def start_writes(count, pos):
                return lax.fori_loop(0, count, lambda _, pos: start_write(pos), pos)

            def read_phase(batch_sems, sems):
                def read(slabs, j, count, sem):
                    rows = pl.ds(pl.multiple_of(j * _PIECE, _PIECE), count * _PIECE)
                    return pltpu.make_async_copy(
                        x_slabs.at[slabs, rows], buf_slabs.at[slabs, rows], sem)

                def band_slabs(band):
                    return pl.ds(band * _BAND, _BAND)

                def start_early(e):
                    band = sum((e >= b * _EARLY_PIECES).astype(jnp.int32) for b in range(1, bands))
                    j = e - band * _EARLY_PIECES
                    k = jnp.maximum(j - first_batch + 2, 0) >> 1
                    read(band_slabs(band), j, 1,
                         batch_sems.at[band * len(_EARLY) + k]).start(priority=1)

                def wait_batch(band, k):
                    sem = batch_sems.at[band * len(_EARLY) + k]

                    @pl.when(k == 0)
                    def _():
                        read(band_slabs(band), 0, first_batch, sem).wait()

                    @pl.when(k > 0)
                    def _():
                        read(band_slabs(band), first_batch + 2 * k - 2, 2, sem).wait()

                def start_small(n, u):
                    band, j = small[u]
                    s = (n >> 1) + 4 * (u % 2)
                    s = jnp.where(s >= _BAND, s - _BAND, s)
                    read(band * _BAND + s, j + (n & 1), 1, sems.at[1]).start()

                w_copy = pltpu.make_async_copy(w_hbm, wbuf, sems.at[0])
                last = [read(band_slabs(band), j, 1, sems.at[2])
                        for j in range(_EARLY_PIECES, _LARGE_PIECES) for band in range(bands)
                        if (j, band) != (_LARGE_PIECES - 1, bands - 1)]
                last.append(read(
                    pl.ds(_SLABS - _BAND, _BAND - _TAIL), _LARGE_PIECES - 1, 1, sems.at[2]))
                tail = read(pl.ds(_SLABS - _TAIL, _TAIL), _LARGE_PIECES - 1, 1, sems.at[3])

                w_copy.start()
                lax.fori_loop(0, _UP_FRONT, lambda e, _: start_early(e), None)

                def idle_slot(n, _):
                    for u in range(len(small)):
                        start_small(n, u)
                        spin(_IDLE_SPINS)

                lax.fori_loop(0, idle_slots, idle_slot, None)
                w_copy.wait()

                def step(n, carry):
                    band, k, s0, started = carry

                    @pl.when(s0 == 0)
                    def _():
                        @pl.when(started < n_early)
                        def _():
                            start_early(started)
                            start_early(started + 1)

                        @pl.when(started == n_early)
                        def _():
                            for copy in last + [tail]:
                                copy.start(priority=1)

                        wait_batch(band, k)

                    ids = iter(range(len(small)))
                    i = _lookup(_EARLY, k)
                    groups = [(band * band_triples + s0 + g, i) for g in range(_STEP_TRIPLES)]
                    blocks = []
                    for c in range(3):
                        start_small(idle_slots + n, next(ids))
                        blocks.append(load(groups, c))
                    xv = jnp.concatenate(blocks, axis=1)
                    for c, stores in enumerate(_STORES):
                        res = dot(xv, wbuf[:, c * 128:(c + 1) * 128])
                        cuts = [p * len(groups) * _GROUP_TILES // stores for p in range(stores + 1)]
                        for lo, hi in zip(cuts, cuts[1:]):
                            start_small(idle_slots + n, next(ids))
                            store(groups, c, res, lo, hi)
                    spin(_PAD_SPINS)

                    started = jnp.where(s0 == 0, started + 2, started)
                    s0 = s0 + _STEP_TRIPLES
                    batch_done = s0 == band_triples
                    k = jnp.where(batch_done, k + 1, k)
                    band_done = k == len(_EARLY)
                    return (jnp.where(band_done, band + 1, band), jnp.where(band_done, 0, k),
                            jnp.where(batch_done, 0, s0), started)

                lax.fori_loop(0, early_steps, step, (zero, zero, zero, jnp.int32(_UP_FRONT)))

                for copy in last:
                    copy.wait()
                lo, hi = map(jnp.int32, _W_EARLY)
                pos = start_writes(_W_FIRST, (zero, lo, lo, hi))
                tail.wait()
                read(slice(None), _LARGE_PIECES, pieces - _LARGE_PIECES,
                     sems.at[1]).wait()
                return pos

            pos = pl.run_scoped(
                read_phase,
                pltpu.SemaphoreType.DMA((n_batches,)),
                pltpu.SemaphoreType.DMA((4,)),
            )

            def step(_, carry):
                pos, s0, q = carry
                for _ in range(_W_PER_STEP):
                    pos = start_write(pos)
                i = _lookup(_LATE, q)
                groups = [(s0 + a, i + b) for a in range(_W_SLABS // 3) for b in range(_LATE_RUN)]
                xv = jnp.concatenate([load(groups, c) for c in range(3)], axis=1)
                res = dot(xv, wbuf[...])
                for c in range(3):
                    store(groups, c, res[:, c * 128:(c + 1) * 128], 0, len(groups) * _GROUP_TILES)
                q = q + 1
                wrap = q == len(_LATE)
                return pos, jnp.where(wrap, s0 + _W_SLABS // 3, s0), jnp.where(wrap, 0, q)

            pos, _, _ = lax.fori_loop(0, late_steps, step, (pos, zero, zero))
            start_writes(n_writes - _W_FIRST - late_steps * _W_PER_STEP, pos)
            pltpu.make_async_copy(buf_slabs, out_slabs, out_sem).wait()

        pl.run_scoped(both_phases, pltpu.SemaphoreType.DMA(()))

    shape = (triples, _GROUPS, group_rows, 128)
    out = pl.pallas_call(
        kernel_function,
        in_specs=[
            pl.BlockSpec(memory_space=pl.ANY),
            pl.BlockSpec(memory_space=pl.ANY),
        ],
        out_specs=pl.BlockSpec(memory_space=pl.ANY),
        out_shape=jax.ShapeDtypeStruct(shape, x.dtype),
        scratch_shapes=[
            pltpu.VMEM(shape, x.dtype),
            pltpu.VMEM((C, C), w.dtype),
            pltpu.SMEM((1,), jnp.int32),
        ],
        compiler_params=pltpu.CompilerParams(
            vmem_limit_bytes=120 * 2**20, disable_bounds_checks=True),
    )(x.reshape(M // 8, 8, 3, 128).transpose(0, 2, 1, 3).reshape(shape), w.reshape(C, C))
    return out.reshape(M // 8, 3, 8, 128).transpose(0, 2, 1, 3).reshape(B, H, W, C)
```
